```python
import os as _os
_os.environ.setdefault("JAX_PLATFORMS", "cpu")
import jax
import jax.numpy as jnp

def _softmax(x, axis=-1):
    return jax.nn.softmax(x, axis=axis)
def _gelu(x):
    return jax.nn.gelu(x, approximate=True)
def _silu(x):
    return jax.nn.silu(x)
def _sigmoid(x):
    return jax.nn.sigmoid(x)
def _layernorm(x, axis=-1, eps=1e-5):
    m = jnp.mean(x, axis=axis, keepdims=True)
    v = jnp.var(x, axis=axis, keepdims=True)
    return (x - m) / jnp.sqrt(v + eps)
def _scatter_add(tgt, idx, src, axis=0):
    return tgt.at[idx].add(src)
def _segment_sum(src, seg, n):
    return jax.ops.segment_sum(src, seg, n)
class _Rng:
    def __init__(self, key):
        self._k = key
    def _next(self):
        self._k, sub = jax.random.split(self._k)
        return sub
    def normal(self, shape):
        return jax.random.normal(self._next(), shape, dtype=jnp.bfloat16)
    def randint(self, lo, hi, shape):
        return jax.random.randint(self._next(), shape, lo, hi, dtype=jnp.int32)
    def uniform(self, shape, lo=0.0, hi=1.0):
        return jax.random.uniform(self._next(), shape, jnp.bfloat16, lo, hi)
    def permutation(self, n):
        return jax.random.permutation(self._next(), n)


kernel_name = 'gated_mix__ssm_conv_s5__geglu_ffn__prompt'

def setup_inputs():
    _rng = _Rng(jax.random.key(int.from_bytes(__import__("os").urandom(4), "little")))
    _w = (lambda a: (lambda t: t.astype(jnp.bfloat16) if jnp.issubdtype(t.dtype, jnp.floating) else t)(jnp.asarray(a)))
    def _A_setup():
        B, S, D = 1, 2048, 512
        P = D
        Lambda_re = -0.5 * jnp.exp((lambda *s: _rng.normal(s) * 0.4)(P))
        Lambda_im = (lambda *s: _rng.normal(s) * 0.4)(P) * 1.0
        B_re = (lambda *s: _rng.normal(s) * 0.4)(P, D) * (D ** -0.5)
        B_im = (lambda *s: _rng.normal(s) * 0.4)(P, D) * (D ** -0.5)
        C_re = (lambda *s: _rng.normal(s) * 0.4)(D, P) * (P ** -0.5)
        C_im = (lambda *s: _rng.normal(s) * 0.4)(D, P) * (P ** -0.5)
        log_dt = (lambda *s: _rng.normal(s) * 0.4)(P) * 0.3 - 2.0
        Dskip = (lambda *s: _rng.normal(s) * 0.4)(D)
        return {
            "x": _w((lambda *s: _rng.normal(s) * 0.05)(B, S, D)),
            "Lambda_re": _w(Lambda_re),
            "Lambda_im": _w(Lambda_im),
            "B_re": _w(B_re),
            "B_im": _w(B_im),
            "C_re": _w(C_re),
            "C_im": _w(C_im),
            "log_dt": _w(log_dt),
            "Dskip": _w(Dskip),
        }
    _A_in = _A_setup()

    def _B_setup():
        B, S, D, F = 1, 2048, 512, 1376
        return {
            "x": _w((lambda *s: _rng.normal(s) * 0.05)(B, S, D)),
            "w_gate": _w((lambda *s: _rng.normal(s) * 0.1)(D, F)),
            "w_up": _w((lambda *s: _rng.normal(s) * 0.1)(D, F)),
            "w_down": _w((lambda *s: _rng.normal(s) * 0.1)(F, D)),
        }
    _B_in = _B_setup()

    return {
        "A_x": _A_in["x"],
        "A_Lambda_re": _A_in["Lambda_re"],
        "A_Lambda_im": _A_in["Lambda_im"],
        "A_B_re": _A_in["B_re"],
        "A_B_im": _A_in["B_im"],
        "A_C_re": _A_in["C_re"],
        "A_C_im": _A_in["C_im"],
        "A_log_dt": _A_in["log_dt"],
        "A_Dskip": _A_in["Dskip"],
        "B_x": _B_in["x"],
        "B_w_gate": _B_in["w_gate"],
        "B_w_up": _B_in["w_up"],
        "B_w_down": _B_in["w_down"],
        "gate_w": _w((lambda *s: _rng.normal(s) * 0.05)(512) * 16.0),
    }

def reference(A_x, A_Lambda_re, A_Lambda_im, A_B_re, A_B_im, A_C_re, A_C_im, A_log_dt, A_Dskip, B_x, B_w_gate, B_w_up, B_w_down, gate_w):
    def _A_ref(x, Lambda_re, Lambda_im, B_re, B_im, C_re, C_im, log_dt, Dskip):
        Bsz, L, H = x.shape
        Lam = Lambda_re + 1j * Lambda_im
        Bmat = B_re + 1j * B_im
        Cmat = C_re + 1j * C_im
        dt = jnp.exp(log_dt)
        Lam_bar = jnp.exp(dt * Lam)
        B_bar = ((Lam_bar - 1.0) / Lam)[:, None] * Bmat
        Bu = jnp.einsum("bld,pd->blp", x + 0j, B_bar)
        h = jnp.zeros_like(Bu[:, 0, :])
        hs = []
        for t in range(L):
            h = Lam_bar[None, :] * h + Bu[:, t, :]
            hs.append(h)
        hseq = jnp.stack(hs, 1)
        y = 2.0 * jnp.einsum("blp,dp->bld", hseq, Cmat).real + x * Dskip[None, None, :]
        return y

    def _B_ref(x, w_gate, w_up, w_down):
        return (_gelu(x @ w_gate) * (x @ w_up)) @ w_down

    x = A_x
    g = _sigmoid((x * gate_w).sum(-1, keepdims=True))
    a = _A_ref(x, A_Lambda_re, A_Lambda_im, A_B_re, A_B_im, A_C_re, A_C_im, A_log_dt, A_Dskip)
    b = _B_ref(x, B_w_gate, B_w_up, B_w_down)
    return g * a + (1 - g) * b
```

```python
import functools
import jax
import jax.numpy as jnp
from jax import lax
import jax.experimental.pallas as pl
import jax.experimental.pallas.tpu as pltpu

S, D, P, F = 2048, 512, 512, 1376
f32, bf16 = jnp.float32, jnp.bfloat16
NT = (((1,), (1,)), ((), ()))


def cmul(ar, ai, br, bi):
    return ar * br - ai * bi, ar * bi + ai * br


def make(M1=256, M2=256, interpret=False):
    NB1, NB2 = S // M1, S // M2

    def kern(x_h, lre_h, lim_h, bre_h, bim_h, cre_h, cim_h, ldt_h, dsk_h, wg_h, wu_h, wd_h, gw_h,
             o_h,
             x_v, lre_v, lim_v, ldt_v, dsk_v, gw_v, b_v, c_raw, c_v, wg_v, wu_v, wd_v, u_v, h_v, o_v, tab,
             sx, sv, sb, sw, so):
        cp = pltpu.make_async_copy
        xc = [cp(x_h.at[pl.ds(j * M1, M1)], x_v.at[pl.ds(j * M1, M1)], sx.at[j]) for j in range(NB1)]
        bc = [cp(bre_h, b_v.at[pl.ds(0, P)], sb.at[0]), cp(bim_h, b_v.at[pl.ds(P, P)], sb.at[1])]
        vc = [cp(s, d, sv.at[i]) for i, (s, d) in enumerate(
            [(lre_h, lre_v), (lim_h, lim_v), (ldt_h, ldt_v), (dsk_h, dsk_v), (gw_h, gw_v)])]
        wc = [cp(cre_h, c_raw.at[0], sw.at[0]), cp(cim_h, c_raw.at[1], sw.at[1]),
              cp(wg_h, wg_v, sw.at[2]), cp(wu_h, wu_v, sw.at[3]), cp(wd_h, wd_v, sw.at[4])]
        for c in vc[:3]:
            c.start()
        xc[0].start()
        for c in bc:
            c.start()
        for c in xc[1:]:
            c.start()
        for c in vc[3:]:
            c.start()
        for c in wc:
            c.start()
        for c in vc[:3]:
            c.wait()
        lre = lre_v[...].astype(f32)
        lim = lim_v[...].astype(f32)
        dt = jnp.exp(ldt_v[...].astype(f32)).astype(bf16).astype(f32)
        mag = jnp.exp(dt * lre)
        ang = dt * lim
        ar, ai = mag * jnp.cos(ang), mag * jnp.sin(ang)
        sc = jnp.maximum(jnp.abs(lre), jnp.abs(lim))
        pr_, pi_ = lre / sc, lim / sc
        den = (pr_ * pr_ + pi_ * pi_) * sc
        nr = ar - 1.0
        kr = (nr * pr_ + ai * pi_) / den
        ki = (ai * pr_ - nr * pi_) / den
        a2r, a2i = cmul(ar, ai, ar, ai)
        a4r, a4i = cmul(a2r, a2i, a2r, a2i)
        row = lax.broadcasted_iota(jnp.int32, (8, P), 0)
        bc8 = lambda v: jnp.broadcast_to(v, (8, P))
        for n, (k, mr, mi) in enumerate([(1, ar, ai), (2, a2r, a2i), (4, a4r, a4i)]):
            tab[2 * n] = jnp.where(row >= k, bc8(mr), 0.0)
            tab[2 * n + 1] = jnp.where(row >= k, bc8(mi), 0.0)
        qr, qi = bc8(ar), bc8(ai)
        for k, mr, mi in [(1, ar, ai), (2, a2r, a2i), (4, a4r, a4i)]:
            tr, ti = cmul(qr, qi, bc8(mr), bc8(mi))
            sel = (row & k) != 0
            qr, qi = jnp.where(sel, tr, qr), jnp.where(sel, ti, qi)
        tab[6] = qr
        tab[7] = qi
        tab[8] = bc8(kr)
        tab[9] = bc8(ki)

        for c in bc:
            c.wait()

        def loop1(j, carry):
            hr_, hi_ = carry
            r0 = pl.multiple_of(j * M1, M1)
            pltpu.make_async_copy(x_h.at[pl.ds(r0, M1)], x_v.at[pl.ds(r0, M1)], sx.at[j]).wait()
            xb = x_v[pl.ds(r0, M1), :]
            u_v[...] = lax.dot_general(xb, b_v[...], NT, preferred_element_type=f32)
            for g in range(M1 // 16):
                outs_r, outs_i = [], []
                for s in range(2):
                    rr = g * 16 + s * 8
                    ur = u_v[rr:rr + 8, 0:P]
                    ui = u_v[rr:rr + 8, P:2 * P]
                    for n, k in enumerate((1, 2, 4)):
                        sr, si = pltpu.roll(ur, k, 0), pltpu.roll(ui, k, 0)
                        mr, mi = tab[2 * n], tab[2 * n + 1]
                        ur, ui = ur + (mr * sr - mi * si), ui + (mr * si + mi * sr)
                    pr, pi = tab[6], tab[7]
                    nhr = ur + (pr * hr_ - pi * hi_)
                    nhi = ui + (pr * hi_ + pi * hr_)
                    hr_ = jnp.broadcast_to(nhr[7:8, :], (8, P))
                    hi_ = jnp.broadcast_to(nhi[7:8, :], (8, P))
                    outs_r.append(nhr)
                    outs_i.append(nhi)
                h_v[pl.ds(r0 + g * 16, 16), 0:P] = jnp.concatenate(outs_r, 0).astype(bf16)
                h_v[pl.ds(r0 + g * 16, 16), P:2 * P] = jnp.concatenate(outs_i, 0).astype(bf16)
            return hr_, hi_

        z = jnp.zeros((8, P), f32)
        lax.fori_loop(0, NB1, loop1, (z, z))

        for c in vc[3:]:
            c.wait()
        for c in wc:
            c.wait()
        kr8, ki8 = tab[8], tab[9]

        def cprep(i, _):
            r = pl.multiple_of(i * 16, 16)
            cr = c_raw[0, pl.ds(r, 16), :].astype(f32)
            ci = c_raw[1, pl.ds(r, 16), :].astype(f32)
            k_r = jnp.concatenate([kr8, kr8], 0)
            k_i = jnp.concatenate([ki8, ki8], 0)
            c_v[pl.ds(r, 16), 0:P] = (2.0 * (cr * k_r - ci * k_i)).astype(bf16)
            c_v[pl.ds(r, 16), P:2 * P] = (-2.0 * (cr * k_i + ci * k_r)).astype(bf16)
            return 0
        lax.fori_loop(0, D // 16, cprep, 0)

        def loop2(j, _):
            r0 = pl.multiple_of(j * M2, M2)
            xb = x_v[pl.ds(r0, M2), :]
            xf = xb.astype(f32)
            zg = jnp.sum(xf * gw_v[...].astype(f32), axis=1, keepdims=True)
            g = jax.nn.sigmoid(zg)
            gt = lax.dot_general(xb, wg_v[...], NT, preferred_element_type=f32)
            up = lax.dot_general(xb, wu_v[...], NT, preferred_element_type=f32)
            act = (jax.nn.gelu(gt, approximate=True) * up).astype(bf16)
            b = jnp.dot(act, wd_v[...], preferred_element_type=f32)
            a = lax.dot_general(h_v[pl.ds(r0, M2), :], c_v[...], NT, preferred_element_type=f32)
            a = a + xf * dsk_v[...].astype(f32)
            o_v[pl.ds(r0, M2), :] = g * a + (1.0 - g) * b
            pltpu.make_async_copy(o_v.at[pl.ds(r0, M2)], o_h.at[pl.ds(r0, M2)], so.at[j]).start()
            return 0
        lax.fori_loop(0, NB2, loop2, 0)
        for j in range(NB2):
            pltpu.make_async_copy(o_v.at[pl.ds(j * M2, M2)], o_h.at[pl.ds(j * M2, M2)], so.at[j]).wait()

    anyspec = pl.BlockSpec(memory_space=pltpu.HBM)
    V = pltpu.VMEM
    call = pl.pallas_call(
        kern,
        out_shape=jax.ShapeDtypeStruct((S, D), f32),
        in_specs=[anyspec] * 13,
        out_specs=anyspec,
        scratch_shapes=[
            V((S, D), bf16), V((1, P), bf16), V((1, P), bf16), V((1, P), bf16), V((1, D), bf16), V((1, D), bf16),
            V((2 * P, D), bf16), V((2, D, P), bf16), V((D, 2 * P), bf16),
            V((F, D), bf16), V((F, D), bf16), V((F, D), bf16),
            V((M1, 2 * P), f32), V((S, 2 * P), bf16), V((S, D), f32), V((10, 8, P), f32),
            pltpu.SemaphoreType.DMA((NB1,)), pltpu.SemaphoreType.DMA((5,)), pltpu.SemaphoreType.DMA((2,)),
            pltpu.SemaphoreType.DMA((5,)), pltpu.SemaphoreType.DMA((NB2,)),
        ],
        compiler_params=pltpu.CompilerParams(vmem_limit_bytes=100 * 1024 * 1024),
    )

    @jax.jit
    def fn(A_x, A_Lambda_re, A_Lambda_im, A_B_re, A_B_im, A_C_re, A_C_im, A_log_dt, A_Dskip,
           B_x, B_w_gate, B_w_up, B_w_down, gate_w):
        r = lambda v: v.reshape(1, -1)
        out = call(A_x.reshape(S, D), r(A_Lambda_re), r(A_Lambda_im), A_B_re, A_B_im, A_C_re, A_C_im,
                   r(A_log_dt), r(A_Dskip), B_w_gate.T, B_w_up.T, B_w_down, r(gate_w))
        return out.reshape(1, S, D)
    return fn


_impl = make(M1=256, M2=256)


def pallas_gated_mix__ssm_conv_s5__geglu_ffn__prompt_kernel(
    A_x, A_Lambda_re, A_Lambda_im, A_B_re, A_B_im, A_C_re, A_C_im, A_log_dt, A_Dskip,
    B_x, B_w_gate, B_w_up, B_w_down, gate_w,
):
    return _impl(A_x, A_Lambda_re, A_Lambda_im, A_B_re, A_B_im, A_C_re, A_C_im, A_log_dt, A_Dskip,
                 B_x, B_w_gate, B_w_up, B_w_down, gate_w)


pallas_gated_mix__ssm_conv_s5__geglu_ffn__prompt_kernel = jax.jit(
    pallas_gated_mix__ssm_conv_s5__geglu_ffn__prompt_kernel)
```

```python
import jax
import jax.numpy as jnp
from jax import lax
import jax.experimental.pallas as pl
import jax.experimental.pallas.tpu as pltpu

S, D, P, F = 2048, 512, 512, 1376
f32, bf16 = jnp.float32, jnp.bfloat16
NT = (((1,), (1,)), ((), ()))


def cmul(ar, ai, br, bi):
    return ar * br - ai * bi, ar * bi + ai * br


def make(M1=256, M2=256, FCH=256, inter=True, sched=None, n2=None, XB=256, cp_at=None, flags=None, pin=True, gs=None, DN=4, YN=1, NBT=8, disc_at=1, first_pieces=8, order=None, now=False, n1=None, xsplit=(256, 512, 1024), plan=(('p', 256), ('d', 256, 1, 0), ('d', 256, 2, 0), ('d', 256, 4, 128)), unroll=1, gpin=1, CPR=32):
    NB1, NB2, NX = S // M1, S // M2, S // XB
    chunks = [(c, min(c + FCH, F)) for c in range(0, F, FCH)]

    def kern(x_h, lre_h, lim_h, bre_h, bim_h, cre_h, cim_h, ldt_h, dsk_h, wg_h, wu_h, wd_h, gw_h,
             o_h,
             x_v, lre_v, lim_v, ldt_v, dsk_v, gw_v, b_v, c_raw, c_v, wg_v, wu_v, wd_v, u_v, h_v, act_v, o_v, tab, zs, g_v,
             sin, so):
        cp = pltpu.make_async_copy
        zs[0] = 0
        XS = [0] + list(xsplit) + [S]
        NXP = len(XS) - 1
        BT = 2 * P // NBT
        xc = [cp(x_h.at[pl.ds(XS[j], XS[j + 1] - XS[j])], x_v.at[pl.ds(XS[j], XS[j + 1] - XS[j])], sin.at[j])
              for j in range(NXP)]
        bc = [cp((bre_h if n * BT < P else bim_h).at[pl.ds(n * BT % P, BT)], b_v.at[pl.ds(n * BT, BT)],
                 sin.at[NXP + n]) for n in range(NBT)]
        s_v, s_c, s_w = NXP + NBT, NXP + NBT + 1, NXP + NBT + 2
        vc = [cp(s_, d_, sin.at[s_v]) for s_, d_ in
              [(lre_h, lre_v), (lim_h, lim_v), (ldt_h, ldt_v), (dsk_h, dsk_v), (gw_h, gw_v)]]
        wc = [cp(cre_h, c_raw.at[0], sin.at[s_c]), cp(cim_h, c_raw.at[1], sin.at[s_c]),
              cp(wg_h, wg_v, sin.at[s_w]), cp(wu_h, wu_v, sin.at[s_w]), cp(wd_h, wd_v, sin.at[s_w])]
        named = {"x": xc, "b": bc, "v": vc, "w": wc}
        started, waited = set(), set()

        def start(k, i):
            if (k, i) not in started:
                started.add((k, i))
                if now and k == "w":
                    return
                named[k][i].start()

        def wait(k, i):
            assert (k, i) in started
            if (k, i) not in waited:
                waited.add((k, i))
                if now and k == "w":
                    return
                named[k][i].wait()

        dflt = ([("v", i) for i in range(5)] + [("x", 0)] + [("b", n) for n in range(NBT)]
                + [("x", j) for j in range(1, NXP)] + [("w", i) for i in range(5)])
        for k, i in (order if order is not None else dflt):
            start(k, i)

        def discretise():
            for i in range(5):
                wait("v", i)
            lre = lre_v[...].astype(f32).reshape(1, P)
            lim = lim_v[...].astype(f32).reshape(1, P)
            dt = jnp.exp(ldt_v[...].astype(f32).reshape(1, P)).astype(bf16).astype(f32)
            mag = jnp.exp(dt * lre)
            ang = dt * lim
            ar, ai = mag * jnp.cos(ang), mag * jnp.sin(ang)
            sc = jnp.maximum(jnp.abs(lre), jnp.abs(lim))
            pr_, pi_ = lre / sc, lim / sc
            den = (pr_ * pr_ + pi_ * pi_) * sc
            nr = ar - 1.0
            kr = (nr * pr_ + ai * pi_) / den
            ki = (ai * pr_ - nr * pi_) / den
            a2r, a2i = cmul(ar, ai, ar, ai)
            a4r, a4i = cmul(a2r, a2i, a2r, a2i)
            row = lax.broadcasted_iota(jnp.int32, (8, P), 0)
            bc8 = lambda v: jnp.broadcast_to(v, (8, P))
            for n, (k, mr, mi) in enumerate([(1, ar, ai), (2, a2r, a2i), (4, a4r, a4i)]):
                tab[2 * n] = jnp.where(row >= k, bc8(mr), 0.0)
                tab[2 * n + 1] = jnp.where(row >= k, bc8(mi), 0.0)
            qr, qi = bc8(ar), bc8(ai)
            for k, mr, mi in [(1, ar, ai), (2, a2r, a2i), (4, a4r, a4i)]:
                tr, ti = cmul(qr, qi, bc8(mr), bc8(mi))
                sel = (row & k) != 0
                qr, qi = jnp.where(sel, tr, qr), jnp.where(sel, ti, qi)
            tab[6] = qr
            tab[7] = qi
            tab[8] = bc8(2.0 * kr)
            tab[9] = bc8(2.0 * ki)

        def cprep(rs, n):
            for r in range(0, n, 16):
                k_r = jnp.concatenate([tab[8], tab[8]], 0)
                k_i = jnp.concatenate([tab[9], tab[9]], 0)
                ri = pl.multiple_of(rs + r, 16) if not isinstance(rs, int) else rs + r
                cr = c_raw[0, pl.ds(ri, 16), :].astype(f32)
                ci = c_raw[1, pl.ds(ri, 16), :].astype(f32)
                ro = pl.multiple_of(zs[0] + rs + r, 16)
                c_v[pl.ds(ro, 16), 0:P] = (cr * k_r - ci * k_i).astype(bf16)
                c_v[pl.ds(ro, 16), P:2 * P] = (-(cr * k_i + ci * k_r)).astype(bf16)

        discretise()
        cdone = 0
        r1 = 0
        cw = False
        for item in plan:
            kind, m = item[0], item[1]
            cnt = item[2] if len(item) > 2 else 1
            crows = item[3] if len(item) > 3 else 0
            r0_, r1 = r1, r1 + m * cnt
            for jj in range(NXP):
                if XS[jj] < r1:
                    wait("x", jj)
            if crows and not cw:
                wait("w", 0)
                wait("w", 1)
                cw = True
            if kind == 'p':
                pw = 2 * P // first_pieces
                xb = x_v[r0_:r1, :]
                for q in range(first_pieces):
                    for n in range(q * pw // BT, -(-(q + 1) * pw // BT)):
                        wait("b", n)
                    u_v[r0_:r1, q * pw:(q + 1) * pw] = lax.dot_general(
                        xb, b_v[q * pw:(q + 1) * pw, :], NT, preferred_element_type=f32)
                continue
            c0_ = cdone

            def blk(i, _, r0_=r0_, m=m, crows=crows, c0_=c0_):
                rr = pl.multiple_of(r0_ + i * m, m) if not isinstance(i, int) else r0_ + i * m
                xb = x_v[pl.ds(rr, m), :]
                if not crows:
                    u_v[pl.ds(rr, m), :] = lax.dot_general(xb, b_v[...], NT, preferred_element_type=f32)
                    return 0
                for q in range(4):
                    res = lax.dot_general(xb, b_v[q * 256:(q + 1) * 256, :], NT, preferred_element_type=f32)
                    u_v[pl.ds(rr, m), q * 256:(q + 1) * 256] = res
                    c_v[D:D + 16, 0:128] = res[m - 16:m, 128:256].astype(bf16)
                    cprep(c0_ + i * crows + q * (crows // 4), crows // 4)
                return 0

            if cnt == 1:
                blk(0, 0)
            else:
                lax.fori_loop(0, cnt, blk, 0)
            cdone += crows * cnt
        assert r1 == S
        for i in range(NXP):
            wait("x", i)
        for i in range(5):
            start("v", i)
            start("w", i)
        for i in range(5):
            wait("v", i)
            wait("w", i)
        if cdone < D:
            cprep(cdone, D - cdone)

        def scan16(r0, g, hr_, hi_):
            outs_r, outs_i = [], []
            for s in range(2):
                rr = pl.multiple_of(r0 + (g * 16 + s * 8), 8)
                ur = u_v[pl.ds(rr, 8), 0:P]
                ui = u_v[pl.ds(rr, 8), P:2 * P]
                for n, k in enumerate((1, 2, 4)):
                    sr, si = pltpu.roll(ur, k, 0), pltpu.roll(ui, k, 0)
                    mr, mi = tab[2 * n], tab[2 * n + 1]
                    ur, ui = ur + (mr * sr - mi * si), ui + (mr * si + mi * sr)
                pr, pi = tab[6], tab[7]
                nhr = ur + (pr * hr_ - pi * hi_)
                nhi = ui + (pr * hi_ + pi * hr_)
                hr_ = jnp.broadcast_to(nhr[7:8, :], (8, P))
                hi_ = jnp.broadcast_to(nhi[7:8, :], (8, P))
                outs_r.append(nhr)
                outs_i.append(nhi)
            ro = pl.multiple_of(zs[0] + g * 16, 16) if pin else g * 16
            h_v[pl.ds(ro, 16), 0:P] = jnp.concatenate(outs_r, 0).astype(bf16)
            h_v[pl.ds(ro, 16), P:2 * P] = jnp.concatenate(outs_i, 0).astype(bf16)
            return hr_, hi_

        def loop2(j, carry):
            hr_, hi_ = carry
            r0 = pl.multiple_of(j * M2, M2)
            NG = M2 // 16
            xb = x_v[pl.ds(r0, M2), :]
            gi = 0
            npc = len(chunks) + DN
            gcount = gs if gs is not None else [2, 2, 2, 2, 2, 1, 1, 1, 1, 2]
            assert len(gcount) == npc and sum(gcount) == NG
            dsl = 16
            pi_ = 0

            def emit(n, hr_, hi_, gi):
                for _ in range(n):
                    hr_, hi_ = scan16(r0, gi, hr_, hi_)
                    gi += 1
                return hr_, hi_, gi

            def pinstore(v):
                if pin:
                    h_v[M2:M2 + 16, 0:128] = v

            def gate_piece(k, nk):
                rows = M2 // nk
                ro = pl.multiple_of(zs[0] + k * rows, 8) if gpin else k * rows
                xs = x_v[pl.ds(r0 + k * rows, rows), :].astype(f32)
                zg = jnp.sum(xs * gw_v[...].astype(f32).reshape(1, D), axis=1, keepdims=True)
                g_v[pl.ds(ro, rows), :] = jnp.broadcast_to(jax.nn.sigmoid(zg), (rows, 128))

            for (c0, c1) in chunks:
                hr_, hi_, gi = emit(gcount[pi_], hr_, hi_, gi)
                pi_ += 1
                gt = lax.dot_general(xb, wg_v[c0:c1, :], NT, preferred_element_type=f32)
                up = lax.dot_general(xb, wu_v[c0:c1, :], NT, preferred_element_type=f32)
                act = (jax.nn.gelu(gt, approximate=True) * up).astype(bf16)
                act_v[:, c0:c1] = act
                w = c1 - c0
                if pi_ <= 4:
                    gate_piece(pi_ - 1, 4)
                if gpin and w >= 128:
                    g_v[M2:M2 + 8, :] = gt[M2 - 8:M2, (w // 128 - 1) * 128:(w // 128) * 128]
                if w >= 128:
                    pinstore(act[M2 - 16:M2, (w // 128 - 1) * 128:(w // 128) * 128])
                else:
                    if pin:
                        h_v[M2:M2 + 16, 0:w] = act[M2 - 16:M2, :]
            xf = xb.astype(f32)
            bs = []
            wn = D // DN
            for n in range(DN):
                hr_, hi_, gi = emit(gcount[pi_], hr_, hi_, gi)
                pi_ += 1
                bn = jnp.dot(act_v[...], wd_v[:, n * wn:(n + 1) * wn], preferred_element_type=f32)
                bs.append(bn)
                pinstore(bn[M2 - 16:M2, wn - 128:wn].astype(bf16))
            b = jnp.concatenate(bs, axis=1) if DN > 1 else bs[0]
            g = g_v[0:M2, :]
            dsk = dsk_v[...].astype(f32).reshape(1, D)
            yw = D // YN
            hb = h_v[0:M2, :]
            for n in range(YN):
                cs = slice(n * yw, (n + 1) * yw)
                a = lax.dot_general(hb, c_v[n * yw:(n + 1) * yw, :], NT, preferred_element_type=f32)
                a = a + xf[:, cs] * dsk[:, cs]
                gg = jnp.concatenate([g] * (yw // 128), axis=1) if yw > 128 else g
                o_v[pl.ds(r0, M2), cs] = gg * a + (1.0 - gg) * b[:, cs]
                pltpu.make_async_copy(o_v.at[pl.ds(r0, M2), pl.ds(n * yw, yw)],
                                      o_h.at[pl.ds(r0, M2), pl.ds(n * yw, yw)], so.at[0]).start()
            return hr_, hi_

        z = jnp.zeros((8, P), f32)
        lax.fori_loop(0, NB2 if n2 is None else n2, loop2, (z, z), unroll=unroll)
        yw = D // YN
        for j in range(NB2 if n2 is None else n2):
            for n in range(YN):
                pltpu.make_async_copy(o_v.at[pl.ds(j * M2, M2), pl.ds(n * yw, yw)],
                                      o_h.at[pl.ds(j * M2, M2), pl.ds(n * yw, yw)], so.at[0]).wait()

    hbm = pl.BlockSpec(memory_space=pltpu.HBM)
    V = pltpu.VMEM
    call = pl.pallas_call(
        kern,
        out_shape=jax.ShapeDtypeStruct((S, D), f32),
        in_specs=[hbm] * 13,
        out_specs=hbm,
        scratch_shapes=[
            V((S, D), bf16), V((P,), bf16), V((P,), bf16), V((P,), bf16), V((D,), bf16), V((D,), bf16),
            V((2 * P, D), bf16), V((2, D, P), bf16), V((D + 16, 2 * P), bf16),
            V((F, D), bf16), V((F, D), bf16), V((F, D), bf16),
            V((S, 2 * P), f32), V((M2 + 16, 2 * P), bf16), V((M2, F), bf16), V((S, D), f32), V((10, 8, P), f32), pltpu.SMEM((1,), jnp.int32), V((M2 + 8, 128), f32),
            pltpu.SemaphoreType.DMA((len(xsplit) + 1 + NBT + 3,)), pltpu.SemaphoreType.DMA((1,)),
        ],
        compiler_params=pltpu.CompilerParams(vmem_limit_bytes=100 * 1024 * 1024, flags=flags),
    )

    @jax.jit
    def fn(A_x, A_Lambda_re, A_Lambda_im, A_B_re, A_B_im, A_C_re, A_C_im, A_log_dt, A_Dskip,
           B_x, B_w_gate, B_w_up, B_w_down, gate_w):
        out = call(A_x.reshape(S, D), A_Lambda_re, A_Lambda_im, A_B_re, A_B_im, A_C_re, A_C_im,
                   A_log_dt, A_Dskip, B_w_gate.T, B_w_up.T, B_w_down, gate_w)
        return out.reshape(1, S, D)
    return fn
SA = {-1: [("x", 1)], 0: [("x", 2), ("w", 0), ("w", 1)], 1: [("x", 3), ("w", 2)], 2: [("x", 4)], 3: [("x", 5), ("w", 3)], 4: [("x", 6), ("v", 3), ("v", 4)], 5: [("x", 7), ("w", 4)]}

LP = {"XLA_TPU_FORCE_LP_LLO_SCHEDULER": True}
ED = {"XLA_TPU_EVENLY_DISTRIBUTE_CRITICAL_NODES": True}

G0 = [2,2,2,2,2,1,2,2,1,0]
PA = (('p', 256), ('d', 256, 1, 0), ('d', 256, 2, 0), ('d', 256, 4, 128))
PB = (('p', 256), ('d', 256, 1, 0), ('d', 512, 1, 0), ('d', 512, 2, 256))
PC = (('p', 256), ('d', 256, 3, 0), ('d', 256, 4, 128))
PD = (('p', 256), ('d', 256, 1, 0), ('d', 512, 1, 0), ('d', 1024, 1, 512))
PE = (('p', 512), ('d', 512, 1, 0), ('d', 512, 2, 256))
G1 = [4,3,3,3,2,1,0]
G2 = [3,3,3,3,2,1,1,0,0,0]
PF = (('p', 256), ('d', 256, 1, 0), ('d', 512, 3, 0))
PG = (('p', 256), ('d', 256, 1, 0), ('d', 512, 1, 0), ('d', 256, 4, 128))
PH = (('p', 256), ('d', 768, 1, 0), ('d', 512, 2, 256))


_impl = make(gs=G1,DN=1,first_pieces=4,YN=4,NBT=4,plan=PB)


def pallas_gated_mix__ssm_conv_s5__geglu_ffn__prompt_kernel(
    A_x, A_Lambda_re, A_Lambda_im, A_B_re, A_B_im, A_C_re, A_C_im, A_log_dt, A_Dskip,
    B_x, B_w_gate, B_w_up, B_w_down, gate_w,
):
    return _impl(A_x, A_Lambda_re, A_Lambda_im, A_B_re, A_B_im, A_C_re, A_C_im, A_log_dt, A_Dskip,
                 B_x, B_w_gate, B_w_up, B_w_down, gate_w)


pallas_gated_mix__ssm_conv_s5__geglu_ffn__prompt_kernel = jax.jit(
    pallas_gated_mix__ssm_conv_s5__geglu_ffn__prompt_kernel)
```

```python
import jax
import jax.numpy as jnp
from jax import lax
import jax.experimental.pallas as pl
import jax.experimental.pallas.tpu as pltpu

S, D, P, F = 2048, 512, 512, 1376
M2 = 256
FCH = 256
X_SPLITS = (0, 256, 512, 1024, S)
B_PIECES = 4
SCAN_GROUPS = (3, 3, 3, 3, 3, 1)
F_CHUNKS = tuple((c, min(c + FCH, F)) for c in range(0, F, FCH))
assert len(SCAN_GROUPS) == len(F_CHUNKS) and sum(SCAN_GROUPS) == M2 // 16

f32, bf16 = jnp.float32, jnp.bfloat16
NT = (((1,), (1,)), ((), ()))


def _cmul(ar, ai, br, bi):
    return ar * br - ai * bi, ar * bi + ai * br


def _kernel(x_h, lre_h, lim_h, bre_h, bim_h, cre_h, cim_h, ldt_h, dsk_h, wg_h, wu_h, wd_h, gw_h,
            o_h,
            x_v, lre_v, lim_v, ldt_v, dsk_v, gw_v, b_v, c_raw, c_v, wg_v, wu_v, wd_v,
            u_v, h_v, act_v, g_v, o_v, tab, zero_s, sem_in, sem_out):
    copy = pltpu.make_async_copy
    zero_s[0] = 0

    nx = len(X_SPLITS) - 1
    brows = 2 * P // B_PIECES
    s_vec, s_c, s_w = nx + B_PIECES, nx + B_PIECES + 1, nx + B_PIECES + 2
    x_cp = [copy(x_h.at[pl.ds(X_SPLITS[j], X_SPLITS[j + 1] - X_SPLITS[j])],
                 x_v.at[pl.ds(X_SPLITS[j], X_SPLITS[j + 1] - X_SPLITS[j])], sem_in.at[j])
            for j in range(nx)]
    b_cp = [copy((bre_h if n * brows < P else bim_h).at[pl.ds(n * brows % P, brows)],
                 b_v.at[pl.ds(n * brows, brows)], sem_in.at[nx + n])
            for n in range(B_PIECES)]
    vec_cp = [copy(src, dst, sem_in.at[s_vec]) for src, dst in
              ((lre_h, lre_v), (lim_h, lim_v), (ldt_h, ldt_v), (dsk_h, dsk_v), (gw_h, gw_v))]
    c_cp = [copy(cre_h, c_raw.at[0], sem_in.at[s_c]), copy(cim_h, c_raw.at[1], sem_in.at[s_c])]
    w_cp = [copy(wg_h, wg_v, sem_in.at[s_w]), copy(wu_h, wu_v, sem_in.at[s_w]),
            copy(wd_h, wd_v, sem_in.at[s_w])]
    for c in vec_cp + x_cp[:1] + b_cp + x_cp[1:] + c_cp + w_cp:
        c.start()

    for c in vec_cp:
        c.wait()
    lre = lre_v[...].astype(f32).reshape(1, P)
    lim = lim_v[...].astype(f32).reshape(1, P)
    dt = jnp.exp(ldt_v[...].astype(f32).reshape(1, P)).astype(bf16).astype(f32)
    mag = jnp.exp(dt * lre)
    ang = dt * lim
    ar, ai = mag * jnp.cos(ang), mag * jnp.sin(ang)
    sc = jnp.maximum(jnp.abs(lre), jnp.abs(lim))
    pr_, pi_ = lre / sc, lim / sc
    den = (pr_ * pr_ + pi_ * pi_) * sc
    nr = ar - 1.0
    kr = (nr * pr_ + ai * pi_) / den
    ki = (ai * pr_ - nr * pi_) / den
    a2r, a2i = _cmul(ar, ai, ar, ai)
    a4r, a4i = _cmul(a2r, a2i, a2r, a2i)
    row = lax.broadcasted_iota(jnp.int32, (8, P), 0)

    def rows8(v):
        return jnp.broadcast_to(v, (8, P))

    powers = ((1, ar, ai), (2, a2r, a2i), (4, a4r, a4i))
    for n, (k, mr, mi) in enumerate(powers):
        tab[2 * n] = jnp.where(row >= k, rows8(mr), 0.0)
        tab[2 * n + 1] = jnp.where(row >= k, rows8(mi), 0.0)
    qr, qi = rows8(ar), rows8(ai)
    for k, mr, mi in powers:
        tr, ti = _cmul(qr, qi, rows8(mr), rows8(mi))
        sel = (row & k) != 0
        qr, qi = jnp.where(sel, tr, qr), jnp.where(sel, ti, qi)
    tab[6] = qr
    tab[7] = qi
    tab[8] = rows8(2.0 * kr)
    tab[9] = rows8(2.0 * ki)

    def c_prep(start, n):
        for r in range(start, start + n, 16):
            k_r = jnp.concatenate([tab[8], tab[8]], 0)
            k_i = jnp.concatenate([tab[9], tab[9]], 0)
            cr = c_raw[0, r:r + 16, :].astype(f32)
            ci = c_raw[1, r:r + 16, :].astype(f32)
            ro = pl.multiple_of(zero_s[0] + r, 16)
            c_v[pl.ds(ro, 16), 0:P] = (cr * k_r - ci * k_i).astype(bf16)
            c_v[pl.ds(ro, 16), P:2 * P] = (-(cr * k_i + ci * k_r)).astype(bf16)

    x_cp[0].wait()
    r0, r1 = X_SPLITS[0], X_SPLITS[1]
    xb = x_v[r0:r1, :]
    for n in range(B_PIECES):
        b_cp[n].wait()
        u_v[r0:r1, n * brows:(n + 1) * brows] = lax.dot_general(
            xb, b_v[n * brows:(n + 1) * brows, :], NT, preferred_element_type=f32)
    for j in range(1, nx - 1):
        r0, r1 = X_SPLITS[j], X_SPLITS[j + 1]
        x_cp[j].wait()
        u_v[r0:r1, :] = lax.dot_general(x_v[r0:r1, :], b_v[...], NT, preferred_element_type=f32)
    r0, r1 = X_SPLITS[nx - 1], X_SPLITS[nx]
    x_cp[nx - 1].wait()
    for c in c_cp:
        c.wait()
    xb = x_v[r0:r1, :]
    for q in range(4):
        res = lax.dot_general(xb, b_v[q * 256:(q + 1) * 256, :], NT, preferred_element_type=f32)
        u_v[r0:r1, q * 256:(q + 1) * 256] = res
        c_v[D:D + 16, 0:128] = res[r1 - r0 - 16:r1 - r0, 128:256].astype(bf16)
        c_prep(q * (D // 4), D // 4)
    for c in w_cp:
        c.wait()

    def scan16(r0, g, hr_, hi_):
        outs_r, outs_i = [], []
        for s in range(2):
            rr = pl.multiple_of(r0 + (g * 16 + s * 8), 8)
            ur = u_v[pl.ds(rr, 8), 0:P]
            ui = u_v[pl.ds(rr, 8), P:2 * P]
            for n, k in enumerate((1, 2, 4)):
                sr, si = pltpu.roll(ur, k, 0), pltpu.roll(ui, k, 0)
                mr, mi = tab[2 * n], tab[2 * n + 1]
                ur, ui = ur + (mr * sr - mi * si), ui + (mr * si + mi * sr)
            pr, pi = tab[6], tab[7]
            nhr = ur + (pr * hr_ - pi * hi_)
            nhi = ui + (pr * hi_ + pi * hr_)
            hr_ = jnp.broadcast_to(nhr[7:8, :], (8, P))
            hi_ = jnp.broadcast_to(nhi[7:8, :], (8, P))
            outs_r.append(nhr)
            outs_i.append(nhi)
        ro = pl.multiple_of(zero_s[0] + g * 16, 16)
        h_v[pl.ds(ro, 16), 0:P] = jnp.concatenate(outs_r, 0).astype(bf16)
        h_v[pl.ds(ro, 16), P:2 * P] = jnp.concatenate(outs_i, 0).astype(bf16)
        return hr_, hi_

    def block(j, carry):
        hr_, hi_ = carry
        r0 = pl.multiple_of(j * M2, M2)
        xb = x_v[pl.ds(r0, M2), :]
        g = 0
        for i, (c0, c1) in enumerate(F_CHUNKS):
            for _ in range(SCAN_GROUPS[i]):
                hr_, hi_ = scan16(r0, g, hr_, hi_)
                g += 1
            gt = lax.dot_general(xb, wg_v[c0:c1, :], NT, preferred_element_type=f32)
            up = lax.dot_general(xb, wu_v[c0:c1, :], NT, preferred_element_type=f32)
            act = (jax.nn.gelu(gt, approximate=True) * up).astype(bf16)
            act_v[:, c0:c1] = act
            w = c1 - c0
            if i < 4:
                rows = M2 // 4
                xs = x_v[pl.ds(r0 + i * rows, rows), :].astype(f32)
                z = jnp.sum(xs * gw_v[...].astype(f32).reshape(1, D), axis=1, keepdims=True)
                g_v[pl.ds(i * rows, rows), :] = jnp.broadcast_to(jax.nn.sigmoid(z), (rows, 128))
            if w >= 128:
                h_v[M2:M2 + 16, 0:128] = act[M2 - 16:M2, (w // 128 - 1) * 128:(w // 128) * 128]
            else:
                h_v[M2:M2 + 16, 0:w] = act[M2 - 16:M2, :]
        xf = xb.astype(f32)
        b = jnp.dot(act_v[...], wd_v[...], preferred_element_type=f32)
        h_v[M2:M2 + 16, 0:128] = b[M2 - 16:M2, D - 128:D].astype(bf16)
        gate = g_v[...]
        dsk = dsk_v[...].astype(f32).reshape(1, D)
        hb = h_v[0:M2, :]
        for n in range(D // 128):
            cs = slice(n * 128, (n + 1) * 128)
            a = lax.dot_general(hb, c_v[n * 128:(n + 1) * 128, :], NT, preferred_element_type=f32)
            a = a + xf[:, cs] * dsk[:, cs]
            o_v[pl.ds(r0, M2), cs] = gate * a + (1.0 - gate) * b[:, cs]
            copy(o_v.at[pl.ds(r0, M2), pl.ds(n * 128, 128)],
                 o_h.at[pl.ds(r0, M2), pl.ds(n * 128, 128)], sem_out.at[0]).start()
        return hr_, hi_

    zeros = jnp.zeros((8, P), f32)
    lax.fori_loop(0, S // M2, block, (zeros, zeros))
    copy(o_v, o_h, sem_out.at[0]).wait()


@jax.jit
def pallas_gated_mix__ssm_conv_s5__geglu_ffn__prompt_kernel(
    A_x: jax.Array,
    A_Lambda_re: jax.Array,
    A_Lambda_im: jax.Array,
    A_B_re: jax.Array,
    A_B_im: jax.Array,
    A_C_re: jax.Array,
    A_C_im: jax.Array,
    A_log_dt: jax.Array,
    A_Dskip: jax.Array,
    B_x: jax.Array,
    B_w_gate: jax.Array,
    B_w_up: jax.Array,
    B_w_down: jax.Array,
    gate_w: jax.Array,
):
    del B_x
    hbm = pl.BlockSpec(memory_space=pltpu.HBM)
    vmem = pltpu.VMEM
    out = pl.pallas_call(
        _kernel,
        out_shape=jax.ShapeDtypeStruct((S, D), f32),
        in_specs=[hbm] * 13,
        out_specs=hbm,
        scratch_shapes=[
            vmem((S, D), bf16),
            vmem((P,), bf16), vmem((P,), bf16), vmem((P,), bf16),
            vmem((D,), bf16), vmem((D,), bf16),
            vmem((2 * P, D), bf16),
            vmem((2, D, P), bf16),
            vmem((D + 16, 2 * P), bf16),
            vmem((F, D), bf16), vmem((F, D), bf16), vmem((F, D), bf16),
            vmem((S, 2 * P), f32),
            vmem((M2 + 16, 2 * P), bf16),
            vmem((M2, F), bf16),
            vmem((M2, 128), f32),
            vmem((S, D), f32),
            vmem((10, 8, P), f32),
            pltpu.SMEM((1,), jnp.int32),
            pltpu.SemaphoreType.DMA((len(X_SPLITS) - 1 + B_PIECES + 3,)),
            pltpu.SemaphoreType.DMA((1,)),
        ],
        compiler_params=pltpu.CompilerParams(vmem_limit_bytes=64 * 1024 * 1024),
    )(A_x.reshape(S, D), A_Lambda_re, A_Lambda_im, A_B_re, A_B_im, A_C_re, A_C_im, A_log_dt,
      A_Dskip, B_w_gate.T, B_w_up.T, B_w_down, gate_w)
    return out.reshape(1, S, D)
```

```python
import jax
import jax.numpy as jnp
from jax import lax
import jax.experimental.pallas as pl
import jax.experimental.pallas.tpu as pltpu

S, D, P, F = 2048, 512, 512, 1376
M2 = 256
FCH = 128
X_SPLITS = (0, 256, 512, 1024, S)
B_PIECES = 4
SCAN_GROUPS = (2, 2, 2, 2, 2, 2, 1, 1, 1, 1, 0)
F_CHUNKS = tuple((c, min(c + FCH, F)) for c in range(0, F, FCH))
assert len(SCAN_GROUPS) == len(F_CHUNKS) and sum(SCAN_GROUPS) == M2 // 16

f32, bf16 = jnp.float32, jnp.bfloat16
NT = (((1,), (1,)), ((), ()))


def _cmul(ar, ai, br, bi):
    return ar * br - ai * bi, ar * bi + ai * br


def _kernel(x_h, lre_h, lim_h, bre_h, bim_h, cre_h, cim_h, ldt_h, dsk_h, wg_h, wu_h, wd_h, gw_h,
            o_h,
            x_v, lre_v, lim_v, ldt_v, dsk_v, gw_v, b_v, c_raw, c_v, wg_v, wu_v, wd_v,
            u_v, h_v, act_v, g_v, o_v, tab, zero_s, sem_in, sem_out):
    copy = pltpu.make_async_copy
    zero_s[0] = 0

    nx = len(X_SPLITS) - 1
    brows = 2 * P // B_PIECES
    s_vec, s_c, s_w = nx + B_PIECES, nx + B_PIECES + 1, nx + B_PIECES + 2
    x_cp = [copy(x_h.at[pl.ds(X_SPLITS[j], X_SPLITS[j + 1] - X_SPLITS[j])],
                 x_v.at[pl.ds(X_SPLITS[j], X_SPLITS[j + 1] - X_SPLITS[j])], sem_in.at[j])
            for j in range(nx)]
    b_cp = [copy((bre_h if n * brows < P else bim_h).at[pl.ds(n * brows % P, brows)],
                 b_v.at[pl.ds(n * brows, brows)], sem_in.at[nx + n])
            for n in range(B_PIECES)]
    vec_cp = [copy(src, dst, sem_in.at[s_vec]) for src, dst in
              ((lre_h, lre_v), (lim_h, lim_v), (ldt_h, ldt_v), (dsk_h, dsk_v), (gw_h, gw_v))]
    c_cp = [copy(cre_h, c_raw.at[0], sem_in.at[s_c]), copy(cim_h, c_raw.at[1], sem_in.at[s_c])]
    w_cp = [copy(wg_h, wg_v, sem_in.at[s_w]), copy(wu_h, wu_v, sem_in.at[s_w]),
            copy(wd_h, wd_v, sem_in.at[s_w])]
    for c in vec_cp + x_cp[:1] + b_cp + x_cp[1:] + c_cp + w_cp:
        c.start()

    for c in vec_cp:
        c.wait()
    lre = lre_v[...].astype(f32).reshape(1, P)
    lim = lim_v[...].astype(f32).reshape(1, P)
    dt = jnp.exp(ldt_v[...].astype(f32).reshape(1, P)).astype(bf16).astype(f32)
    mag = jnp.exp(dt * lre)
    ang = dt * lim
    ar, ai = mag * jnp.cos(ang), mag * jnp.sin(ang)
    sc = jnp.maximum(jnp.abs(lre), jnp.abs(lim))
    pr_, pi_ = lre / sc, lim / sc
    den = (pr_ * pr_ + pi_ * pi_) * sc
    nr = ar - 1.0
    kr = (nr * pr_ + ai * pi_) / den
    ki = (ai * pr_ - nr * pi_) / den
    a2r, a2i = _cmul(ar, ai, ar, ai)
    a4r, a4i = _cmul(a2r, a2i, a2r, a2i)
    row = lax.broadcasted_iota(jnp.int32, (8, P), 0)

    def rows8(v):
        return jnp.broadcast_to(v, (8, P))

    powers = ((1, ar, ai), (2, a2r, a2i), (4, a4r, a4i))
    for n, (k, mr, mi) in enumerate(powers):
        tab[2 * n] = jnp.where(row >= k, rows8(mr), 0.0)
        tab[2 * n + 1] = jnp.where(row >= k, rows8(mi), 0.0)
    qr, qi = rows8(ar), rows8(ai)
    for k, mr, mi in powers:
        tr, ti = _cmul(qr, qi, rows8(mr), rows8(mi))
        sel = (row & k) != 0
        qr, qi = jnp.where(sel, tr, qr), jnp.where(sel, ti, qi)
    tab[6] = qr
    tab[7] = qi
    tab[8] = rows8(2.0 * kr)
    tab[9] = rows8(2.0 * ki)

    def c_prep(start, n):
        for r in range(start, start + n, 16):
            k_r = jnp.concatenate([tab[8], tab[8]], 0)
            k_i = jnp.concatenate([tab[9], tab[9]], 0)
            cr = c_raw[0, r:r + 16, :].astype(f32)
            ci = c_raw[1, r:r + 16, :].astype(f32)
            ro = pl.multiple_of(zero_s[0] + r, 16)
            c_v[pl.ds(ro, 16), 0:P] = (cr * k_r - ci * k_i).astype(bf16)
            c_v[pl.ds(ro, 16), P:2 * P] = (-(cr * k_i + ci * k_r)).astype(bf16)

    x_cp[0].wait()
    r0, r1 = X_SPLITS[0], X_SPLITS[1]
    xb = x_v[r0:r1, :]
    for n in range(B_PIECES):
        b_cp[n].wait()
        u_v[r0:r1, n * brows:(n + 1) * brows] = lax.dot_general(
            xb, b_v[n * brows:(n + 1) * brows, :], NT, preferred_element_type=f32)
    for j in range(1, nx - 1):
        r0, r1 = X_SPLITS[j], X_SPLITS[j + 1]
        x_cp[j].wait()
        u_v[r0:r1, :] = lax.dot_general(x_v[r0:r1, :], b_v[...], NT, preferred_element_type=f32)
    r0, r1 = X_SPLITS[nx - 1], X_SPLITS[nx]
    x_cp[nx - 1].wait()
    for c in c_cp:
        c.wait()
    xb = x_v[r0:r1, :]
    for q in range(4):
        res = lax.dot_general(xb, b_v[q * 256:(q + 1) * 256, :], NT, preferred_element_type=f32)
        u_v[r0:r1, q * 256:(q + 1) * 256] = res
        c_v[D:D + 16, 0:128] = res[r1 - r0 - 16:r1 - r0, 128:256].astype(bf16)
        c_prep(q * (D // 4), D // 4)
    for c in w_cp:
        c.wait()

    def scan16(r0, g, hr_, hi_):
        outs_r, outs_i = [], []
        for s in range(2):
            rr = pl.multiple_of(r0 + (g * 16 + s * 8), 8)
            ur = u_v[pl.ds(rr, 8), 0:P]
            ui = u_v[pl.ds(rr, 8), P:2 * P]
            for n, k in enumerate((1, 2, 4)):
                sr, si = pltpu.roll(ur, k, 0), pltpu.roll(ui, k, 0)
                mr, mi = tab[2 * n], tab[2 * n + 1]
                ur, ui = ur + (mr * sr - mi * si), ui + (mr * si + mi * sr)
            pr, pi = tab[6], tab[7]
            nhr = ur + (pr * hr_ - pi * hi_)
            nhi = ui + (pr * hi_ + pi * hr_)
            hr_ = jnp.broadcast_to(nhr[7:8, :], (8, P))
            hi_ = jnp.broadcast_to(nhi[7:8, :], (8, P))
            outs_r.append(nhr)
            outs_i.append(nhi)
        ro = pl.multiple_of(zero_s[0] + g * 16, 16)
        h_v[pl.ds(ro, 16), 0:P] = jnp.concatenate(outs_r, 0).astype(bf16)
        h_v[pl.ds(ro, 16), P:2 * P] = jnp.concatenate(outs_i, 0).astype(bf16)
        return hr_, hi_

    def block(j, carry):
        hr_, hi_ = carry
        r0 = pl.multiple_of(j * M2, M2)
        xb = x_v[pl.ds(r0, M2), :]
        g = 0
        for i, (c0, c1) in enumerate(F_CHUNKS):
            for _ in range(SCAN_GROUPS[i]):
                hr_, hi_ = scan16(r0, g, hr_, hi_)
                g += 1
            gt = lax.dot_general(xb, wg_v[c0:c1, :], NT, preferred_element_type=f32)
            up = lax.dot_general(xb, wu_v[c0:c1, :], NT, preferred_element_type=f32)
            act = (jax.nn.gelu(gt, approximate=True) * up).astype(bf16)
            act_v[:, c0:c1] = act
            w = c1 - c0
            if i < 4:
                rows = M2 // 4
                xs = x_v[pl.ds(r0 + i * rows, rows), :].astype(f32)
                z = jnp.sum(xs * gw_v[...].astype(f32).reshape(1, D), axis=1, keepdims=True)
                g_v[pl.ds(i * rows, rows), :] = jnp.broadcast_to(jax.nn.sigmoid(z), (rows, 128))
            if w >= 128:
                h_v[M2:M2 + 16, 0:128] = act[M2 - 16:M2, (w // 128 - 1) * 128:(w // 128) * 128]
            else:
                h_v[M2:M2 + 16, 0:w] = act[M2 - 16:M2, :]
        xf = xb.astype(f32)
        b = jnp.dot(act_v[...], wd_v[...], preferred_element_type=f32)
        h_v[M2:M2 + 16, 0:128] = b[M2 - 16:M2, D - 128:D].astype(bf16)
        gate = g_v[...]
        dsk = dsk_v[...].astype(f32).reshape(1, D)
        hb = h_v[0:M2, :]
        for n in range(D // 128):
            cs = slice(n * 128, (n + 1) * 128)
            a = lax.dot_general(hb, c_v[n * 128:(n + 1) * 128, :], NT, preferred_element_type=f32)
            a = a + xf[:, cs] * dsk[:, cs]
            o_v[pl.ds(r0, M2), cs] = gate * a + (1.0 - gate) * b[:, cs]
            copy(o_v.at[pl.ds(r0, M2), pl.ds(n * 128, 128)],
                 o_h.at[pl.ds(r0, M2), pl.ds(n * 128, 128)], sem_out.at[0]).start()
        return hr_, hi_

    zeros = jnp.zeros((8, P), f32)
    lax.fori_loop(0, S // M2, block, (zeros, zeros))
    copy(o_v, o_h, sem_out.at[0]).wait()


@jax.jit
def pallas_gated_mix__ssm_conv_s5__geglu_ffn__prompt_kernel(
    A_x: jax.Array,
    A_Lambda_re: jax.Array,
    A_Lambda_im: jax.Array,
    A_B_re: jax.Array,
    A_B_im: jax.Array,
    A_C_re: jax.Array,
    A_C_im: jax.Array,
    A_log_dt: jax.Array,
    A_Dskip: jax.Array,
    B_x: jax.Array,
    B_w_gate: jax.Array,
    B_w_up: jax.Array,
    B_w_down: jax.Array,
    gate_w: jax.Array,
):
    del B_x
    assert A_x.shape == (1, S, D) and A_B_re.shape == (P, D) and A_C_re.shape == (D, P)
    assert B_w_gate.shape == (D, F) and B_w_up.shape == (D, F) and B_w_down.shape == (F, D)
    hbm = pl.BlockSpec(memory_space=pltpu.HBM)
    vmem = pltpu.VMEM
    out = pl.pallas_call(
        _kernel,
        out_shape=jax.ShapeDtypeStruct((S, D), f32),
        in_specs=[hbm] * 13,
        out_specs=hbm,
        scratch_shapes=[
            vmem((S, D), bf16),
            vmem((P,), bf16), vmem((P,), bf16), vmem((P,), bf16),
            vmem((D,), bf16), vmem((D,), bf16),
            vmem((2 * P, D), bf16),
            vmem((2, D, P), bf16),
            vmem((D + 16, 2 * P), bf16),
            vmem((F, D), bf16), vmem((F, D), bf16), vmem((F, D), bf16),
            vmem((S, 2 * P), f32),
            vmem((M2 + 16, 2 * P), bf16),
            vmem((M2, F), bf16),
            vmem((M2, 128), f32),
            vmem((S, D), f32),
            vmem((10, 8, P), f32),
            pltpu.SMEM((1,), jnp.int32),
            pltpu.SemaphoreType.DMA((len(X_SPLITS) - 1 + B_PIECES + 3,)),
            pltpu.SemaphoreType.DMA((1,)),
        ],
        compiler_params=pltpu.CompilerParams(vmem_limit_bytes=64 * 1024 * 1024),
    )(A_x.reshape(S, D), A_Lambda_re, A_Lambda_im, A_B_re, A_B_im, A_C_re, A_C_im, A_log_dt,
      A_Dskip, B_w_gate.T, B_w_up.T, B_w_down, gate_w)
    return out.reshape(1, S, D)
```

```python
import jax
import jax.numpy as jnp
from jax import lax
import jax.experimental.pallas as pl
import jax.experimental.pallas.tpu as pltpu

S, D, P, F = 2048, 512, 512, 1376
M2 = 256
FCH = 128
X_SPLITS = (0, 256, 512, 1024, S)
B_PIECES = 4
SCAN_GROUPS = (2, 2, 2, 2, 2, 2, 1, 1, 1, 1, 0)
F_CHUNKS = tuple((c, min(c + FCH, F)) for c in range(0, F, FCH))
assert len(SCAN_GROUPS) == len(F_CHUNKS) and sum(SCAN_GROUPS) == M2 // 16

f32, bf16 = jnp.float32, jnp.bfloat16
NT = (((1,), (1,)), ((), ()))


def _cmul(ar, ai, br, bi):
    return ar * br - ai * bi, ar * bi + ai * br


def _kernel(x_h, lre_h, lim_h, bre_h, bim_h, cre_h, cim_h, ldt_h, dsk_h, wg_h, wu_h, wd_h, gw_h,
            o_h,
            x_v, lre_v, lim_v, ldt_v, dsk_v, gw_v, b_v, c_raw, c_v, wg_v, wu_v, wd_v,
            u_v, h_v, act_v, g_v, o_v, tab, zero_s, sem_in, sem_out):
    copy = pltpu.make_async_copy
    zero_s[0] = 0

    nx = len(X_SPLITS) - 1
    brows = 2 * P // B_PIECES
    s_vec, s_c, s_w = nx + B_PIECES, nx + B_PIECES + 1, nx + B_PIECES + 2
    x_cp = [copy(x_h.at[pl.ds(X_SPLITS[j], X_SPLITS[j + 1] - X_SPLITS[j])],
                 x_v.at[pl.ds(X_SPLITS[j], X_SPLITS[j + 1] - X_SPLITS[j])], sem_in.at[j])
            for j in range(nx)]
    b_cp = [copy((bre_h if n * brows < P else bim_h).at[pl.ds(n * brows % P, brows)],
                 b_v.at[pl.ds(n * brows, brows)], sem_in.at[nx + n])
            for n in range(B_PIECES)]
    vec_cp = [copy(src, dst, sem_in.at[s_vec]) for src, dst in
              ((lre_h, lre_v), (lim_h, lim_v), (ldt_h, ldt_v), (dsk_h, dsk_v), (gw_h, gw_v))]
    c_cp = [copy(cre_h, c_raw.at[0], sem_in.at[s_c]), copy(cim_h, c_raw.at[1], sem_in.at[s_c])]
    w_cp = [copy(wg_h, wg_v, sem_in.at[s_w]), copy(wu_h, wu_v, sem_in.at[s_w]),
            copy(wd_h, wd_v, sem_in.at[s_w])]
    for c in vec_cp + x_cp[:1] + b_cp + x_cp[1:] + c_cp + w_cp:
        c.start()

    for c in vec_cp:
        c.wait()
    lre = lre_v[...].astype(f32).reshape(1, P)
    lim = lim_v[...].astype(f32).reshape(1, P)
    dt = jnp.exp(ldt_v[...].astype(f32).reshape(1, P)).astype(bf16).astype(f32)
    mag = jnp.exp(dt * lre)
    ang = dt * lim
    ar, ai = mag * jnp.cos(ang), mag * jnp.sin(ang)
    sc = jnp.maximum(jnp.abs(lre), jnp.abs(lim))
    pr_, pi_ = lre / sc, lim / sc
    den = (pr_ * pr_ + pi_ * pi_) * sc
    nr = ar - 1.0
    kr = (nr * pr_ + ai * pi_) / den
    ki = (ai * pr_ - nr * pi_) / den
    a2r, a2i = _cmul(ar, ai, ar, ai)
    a4r, a4i = _cmul(a2r, a2i, a2r, a2i)
    row = lax.broadcasted_iota(jnp.int32, (8, P), 0)

    def rows8(v):
        return jnp.broadcast_to(v, (8, P))

    powers = ((1, ar, ai), (2, a2r, a2i), (4, a4r, a4i))
    for n, (k, mr, mi) in enumerate(powers):
        tab[2 * n] = jnp.where(row >= k, rows8(mr), 0.0)
        tab[2 * n + 1] = jnp.where(row >= k, rows8(mi), 0.0)
    qr, qi = rows8(ar), rows8(ai)
    for k, mr, mi in powers:
        tr, ti = _cmul(qr, qi, rows8(mr), rows8(mi))
        sel = (row & k) != 0
        qr, qi = jnp.where(sel, tr, qr), jnp.where(sel, ti, qi)
    tab[6] = qr
    tab[7] = qi
    tab[8] = rows8(2.0 * kr)
    tab[9] = rows8(2.0 * ki)

    def c_prep(start, n):
        for r in range(start, start + n, 16):
            k_r = jnp.concatenate([tab[8], tab[8]], 0)
            k_i = jnp.concatenate([tab[9], tab[9]], 0)
            cr = c_raw[0, r:r + 16, :].astype(f32)
            ci = c_raw[1, r:r + 16, :].astype(f32)
            ro = pl.multiple_of(zero_s[0] + r, 16)
            c_v[pl.ds(ro, 16), 0:P] = (cr * k_r - ci * k_i).astype(bf16)
            c_v[pl.ds(ro, 16), P:2 * P] = (-(cr * k_i + ci * k_r)).astype(bf16)

    x_cp[0].wait()
    r0, r1 = X_SPLITS[0], X_SPLITS[1]
    xb = x_v[r0:r1, :]
    for n in range(B_PIECES):
        b_cp[n].wait()
        u_v[r0:r1, n * brows:(n + 1) * brows] = lax.dot_general(
            xb, b_v[n * brows:(n + 1) * brows, :], NT, preferred_element_type=f32)
    for j in range(1, nx - 1):
        r0, r1 = X_SPLITS[j], X_SPLITS[j + 1]
        x_cp[j].wait()
        u_v[r0:r1, :] = lax.dot_general(x_v[r0:r1, :], b_v[...], NT, preferred_element_type=f32)
    r0, r1 = X_SPLITS[nx - 1], X_SPLITS[nx]
    x_cp[nx - 1].wait()
    for c in c_cp:
        c.wait()
    k = 0
    for rr in range(r0, r1, 256):
        xb = x_v[rr:rr + 256, :]
        for q in range(2 * P // 128):
            res = lax.dot_general(xb, b_v[q * 128:(q + 1) * 128, :], NT, preferred_element_type=f32)
            u_v[rr:rr + 256, q * 128:(q + 1) * 128] = res
            c_v[D:D + 16, 0:128] = res[240:256, :].astype(bf16)
            c_prep(k * 16, 16)
            k += 1
    assert k * 16 == D
    for c in w_cp:
        c.wait()

    def scan16(r0, g, hr_, hi_):
        outs_r, outs_i = [], []
        for s in range(2):
            rr = pl.multiple_of(r0 + (g * 16 + s * 8), 8)
            ur = u_v[pl.ds(rr, 8), 0:P]
            ui = u_v[pl.ds(rr, 8), P:2 * P]
            for n, k in enumerate((1, 2, 4)):
                sr, si = pltpu.roll(ur, k, 0), pltpu.roll(ui, k, 0)
                mr, mi = tab[2 * n], tab[2 * n + 1]
                ur, ui = ur + (mr * sr - mi * si), ui + (mr * si + mi * sr)
            pr, pi = tab[6], tab[7]
            nhr = ur + (pr * hr_ - pi * hi_)
            nhi = ui + (pr * hi_ + pi * hr_)
            hr_ = jnp.broadcast_to(nhr[7:8, :], (8, P))
            hi_ = jnp.broadcast_to(nhi[7:8, :], (8, P))
            outs_r.append(nhr)
            outs_i.append(nhi)
        ro = pl.multiple_of(zero_s[0] + g * 16, 16)
        h_v[pl.ds(ro, 16), 0:P] = jnp.concatenate(outs_r, 0).astype(bf16)
        h_v[pl.ds(ro, 16), P:2 * P] = jnp.concatenate(outs_i, 0).astype(bf16)
        return hr_, hi_

    def block(j, carry):
        hr_, hi_ = carry
        r0 = pl.multiple_of(j * M2, M2)
        xb = x_v[pl.ds(r0, M2), :]
        g = 0
        for i, (c0, c1) in enumerate(F_CHUNKS):
            for _ in range(SCAN_GROUPS[i]):
                hr_, hi_ = scan16(r0, g, hr_, hi_)
                g += 1
            gt = lax.dot_general(xb, wg_v[c0:c1, :], NT, preferred_element_type=f32)
            up = lax.dot_general(xb, wu_v[c0:c1, :], NT, preferred_element_type=f32)
            act = (jax.nn.gelu(gt, approximate=True) * up).astype(bf16)
            act_v[:, c0:c1] = act
            w = c1 - c0
            if i < 4:
                rows = M2 // 4
                xs = x_v[pl.ds(r0 + i * rows, rows), :].astype(f32)
                z = jnp.sum(xs * gw_v[...].astype(f32).reshape(1, D), axis=1, keepdims=True)
                g_v[pl.ds(i * rows, rows), :] = jnp.broadcast_to(jax.nn.sigmoid(z), (rows, 128))
            if w >= 128:
                h_v[M2:M2 + 16, 0:128] = act[M2 - 16:M2, (w // 128 - 1) * 128:(w // 128) * 128]
            else:
                h_v[M2:M2 + 16, 0:w] = act[M2 - 16:M2, :]
        xf = xb.astype(f32)
        b = jnp.dot(act_v[...], wd_v[...], preferred_element_type=f32)
        h_v[M2:M2 + 16, 0:128] = b[M2 - 16:M2, D - 128:D].astype(bf16)
        gate = g_v[...]
        dsk = dsk_v[...].astype(f32).reshape(1, D)
        hb = h_v[0:M2, :]
        for n in range(D // 128):
            cs = slice(n * 128, (n + 1) * 128)
            a = lax.dot_general(hb, c_v[n * 128:(n + 1) * 128, :], NT, preferred_element_type=f32)
            a = a + xf[:, cs] * dsk[:, cs]
            o_v[pl.ds(r0, M2), cs] = gate * a + (1.0 - gate) * b[:, cs]
            copy(o_v.at[pl.ds(r0, M2), pl.ds(n * 128, 128)],
                 o_h.at[pl.ds(r0, M2), pl.ds(n * 128, 128)], sem_out.at[0]).start()
        return hr_, hi_

    zeros = jnp.zeros((8, P), f32)
    lax.fori_loop(0, S // M2, block, (zeros, zeros))
    copy(o_v, o_h, sem_out.at[0]).wait()


@jax.jit
def pallas_gated_mix__ssm_conv_s5__geglu_ffn__prompt_kernel(
    A_x: jax.Array,
    A_Lambda_re: jax.Array,
    A_Lambda_im: jax.Array,
    A_B_re: jax.Array,
    A_B_im: jax.Array,
    A_C_re: jax.Array,
    A_C_im: jax.Array,
    A_log_dt: jax.Array,
    A_Dskip: jax.Array,
    B_x: jax.Array,
    B_w_gate: jax.Array,
    B_w_up: jax.Array,
    B_w_down: jax.Array,
    gate_w: jax.Array,
):
    del B_x
    assert A_x.shape == (1, S, D) and A_B_re.shape == (P, D) and A_C_re.shape == (D, P)
    assert B_w_gate.shape == (D, F) and B_w_up.shape == (D, F) and B_w_down.shape == (F, D)
    hbm = pl.BlockSpec(memory_space=pltpu.HBM)
    vmem = pltpu.VMEM
    out = pl.pallas_call(
        _kernel,
        out_shape=jax.ShapeDtypeStruct((S, D), f32),
        in_specs=[hbm] * 13,
        out_specs=hbm,
        scratch_shapes=[
            vmem((S, D), bf16),
            vmem((P,), bf16), vmem((P,), bf16), vmem((P,), bf16),
            vmem((D,), bf16), vmem((D,), bf16),
            vmem((2 * P, D), bf16),
            vmem((2, D, P), bf16),
            vmem((D + 16, 2 * P), bf16),
            vmem((F, D), bf16), vmem((F, D), bf16), vmem((F, D), bf16),
            vmem((S, 2 * P), f32),
            vmem((M2 + 16, 2 * P), bf16),
            vmem((M2, F), bf16),
            vmem((M2, 128), f32),
            vmem((S, D), f32),
            vmem((10, 8, P), f32),
            pltpu.SMEM((1,), jnp.int32),
            pltpu.SemaphoreType.DMA((len(X_SPLITS) - 1 + B_PIECES + 3,)),
            pltpu.SemaphoreType.DMA((1,)),
        ],
        compiler_params=pltpu.CompilerParams(vmem_limit_bytes=64 * 1024 * 1024),
    )(A_x.reshape(S, D), A_Lambda_re, A_Lambda_im, A_B_re, A_B_im, A_C_re, A_C_im, A_log_dt,
      A_Dskip, B_w_gate.T, B_w_up.T, B_w_down, gate_w)
    return out.reshape(1, S, D)
```
